```python
import os as _os
_os.environ.setdefault("JAX_PLATFORMS", "cpu")
import jax
import jax.numpy as jnp

def _softmax(x, axis=-1):
    return jax.nn.softmax(x, axis=axis)
def _gelu(x):
    return jax.nn.gelu(x, approximate=True)
def _silu(x):
    return jax.nn.silu(x)
def _sigmoid(x):
    return jax.nn.sigmoid(x)
def _layernorm(x, axis=-1, eps=1e-5):
    m = jnp.mean(x, axis=axis, keepdims=True)
    v = jnp.var(x, axis=axis, keepdims=True)
    return (x - m) / jnp.sqrt(v + eps)
def _scatter_add(tgt, idx, src, axis=0):
    return tgt.at[idx].add(src)
def _segment_sum(src, seg, n):
    return jax.ops.segment_sum(src, seg, n)
class _Rng:
    def __init__(self, key):
        self._k = key
    def _next(self):
        self._k, sub = jax.random.split(self._k)
        return sub
    def normal(self, shape):
        return jax.random.normal(self._next(), shape, dtype=jnp.bfloat16)
    def randint(self, lo, hi, shape):
        return jax.random.randint(self._next(), shape, lo, hi, dtype=jnp.int32)
    def uniform(self, shape, lo=0.0, hi=1.0):
        return jax.random.uniform(self._next(), shape, jnp.bfloat16, lo, hi)
    def permutation(self, n):
        return jax.random.permutation(self._next(), n)


kernel_name = 'gated_mix__mha_block__ssm_conv_h3__prompt'

def setup_inputs():
    _rng = _Rng(jax.random.key(int.from_bytes(__import__("os").urandom(4), "little")))
    _w = (lambda a: (lambda t: t.astype(jnp.bfloat16) if jnp.issubdtype(t.dtype, jnp.floating) else t)(jnp.asarray(a)))
    def _A_setup():
        B, S, D, H = 1, 2048, 640, 32
        return {
            "x": _w((lambda *s: _rng.normal(s) * 0.05)(B, S, D)),
            "wqkv": _w((lambda *s: _rng.normal(s) * 0.4)(D, 3 * D)),
            "wo": _w((lambda *s: _rng.normal(s) * 0.05)(D, D)),
        }
    _A_in = _A_setup()

    def _B_setup():
        B, S, D = 1, 2048, 640
        ks = 4
        return {
            "q": _w((lambda *s: _rng.normal(s) * 0.05)(B, S, D)),
            "k": _w((lambda *s: _rng.normal(s) * 0.4)(B, S, D)),
            "v": _w((lambda *s: _rng.normal(s) * 0.4)(B, S, D)),
            "shift_k": _w((lambda *s: _rng.normal(s) * 0.4)(D, ks) * 0.5),
            "ssm_k": _w((lambda *s: _rng.normal(s) * 0.4)(D, S) * (1.0 / S ** 0.5)),
            "ssm_D": _w((lambda *s: _rng.normal(s) * 0.4)(D)),
        }
    _B_in = _B_setup()

    return {
        "A_x": _A_in["x"],
        "A_wqkv": _A_in["wqkv"],
        "A_wo": _A_in["wo"],
        "B_q": _B_in["q"],
        "B_k": _B_in["k"],
        "B_v": _B_in["v"],
        "B_shift_k": _B_in["shift_k"],
        "B_ssm_k": _B_in["ssm_k"],
        "B_ssm_D": _B_in["ssm_D"],
        "gate_w": _w((lambda *s: _rng.normal(s) * 0.05)(640) * 16.0),
    }

def reference(A_x, A_wqkv, A_wo, B_q, B_k, B_v, B_shift_k, B_ssm_k, B_ssm_D, gate_w):
    def _A_ref(x, wqkv, wo):
        B, S, D = x.shape
        H = 32
        Dh = D // H
        qkv = (lambda x, *d: x.transpose(*d))((x @ wqkv).reshape(B, S, 3, H, Dh), 2, 0, 3, 1, 4)
        q, k, v = qkv[0], qkv[1], qkv[2]
        scores = jnp.einsum("bhqd,bhkd->bhqk", q, k) * (Dh ** -0.5)
        p = _softmax(scores, axis=-1)
        o = jnp.einsum("bhqk,bhkd->bhqd", p, v)
        return (lambda x, *d: x.transpose(*d))(o, 0, 2, 1, 3).reshape(B, S, D) @ wo

    def _B_ref(q, k, v, shift_k, ssm_k, ssm_D):
        B, S, D = q.shape
        ks = shift_k.shape[-1]
        k_pad = jnp.pad(k, ((0, 0), (ks - 1, 0), (0, 0)))
        k_shift = jnp.zeros_like(k)
        for t in range(ks):
            k_shift = k_shift + k_pad[:, t:t + S, :] * shift_k[:, ks - 1 - t][None, None, :]
        kv = k_shift * v
        L = 2 * S
        kv_pad = jnp.pad(kv, ((0, 0), (0, S), (0, 0)))
        kf_pad = jnp.pad(ssm_k, ((0, 0), (0, S)))
        kv_f = (lambda x, axes=(-2,-1): jnp.fft.rfft2(x.astype(jnp.float32), axes=axes))(kv_pad[:, None, :, :], axes=(1, 2))
        kf_f = (lambda x, axes=(-2,-1): jnp.fft.rfft2(x.astype(jnp.float32), axes=axes))(kf_pad[:, None, :], axes=(1, 2))
        kf_f = (lambda x, *d: x.transpose(*d))(kf_f, 1, 2, 0)
        y_f = kv_f * kf_f[None, :, :, :]
        y = (lambda x, s, axes=(-2,-1): jnp.fft.irfft2(x, s=s, axes=axes).astype(jnp.bfloat16))(y_f, (1, L), axes=(1, 2))[:, 0, :S, :]
        y = y + kv * ssm_D[None, None, :]
        return q * y

    x = A_x
    g = _sigmoid((x * gate_w).sum(-1, keepdims=True))
    a = _A_ref(x, A_wqkv, A_wo)
    b = _B_ref(x, B_k, B_v, B_shift_k, B_ssm_k, B_ssm_D)
    return g * a + (1 - g) * b
```

```python
import numpy as np
import jax
import jax.numpy as jnp
from jax import lax
import jax.experimental.pallas as pl
import jax.experimental.pallas.tpu as pltpu

_H = 32
_QB = 512
_KC = 128
_WIN = 24
_C = 128

_NN = (((1,), (0,)), ((), ()))
_NT = (((1,), (1,)), ((), ()))
_F32 = jnp.float32
_BF16 = jnp.bfloat16


def _dft_matrices():
    theta = 2.0 * np.pi * (np.arange(_C) + 0.5) / (2 * _C)
    ang = theta[:, None] * np.arange(_C)[None, :]
    fwd = np.concatenate([np.cos(ang), -np.sin(ang)], axis=0)
    inv = fwd.T / _C
    return fwd.astype(np.float32), np.ascontiguousarray(inv).astype(np.float32)


def _dot(a, b, dims=_NN):
    return lax.dot_general(a, b, dims, preferred_element_type=_F32)


def _kernel(x_hbm, w_hbm, wo_hbm, bk_hbm, bv_hbm, h_hbm,
            shift_ref, d_ref, gw_ref, fwd_ref, inv_ref,
            out_hbm,
            x_v, w_v, wt_v, wo_v, bk_v, bv_v, h_v,
            k_all, q_all, v_all, s_buf, ot_v,
            kv_v, xf_v, hf_v, yf_v, out_v, sems, osems):
    S, D = x_v.shape
    Dh = D // _H
    NQ = S // _QB
    NK = S // _KC
    NC = S // _C
    NG = D // 128
    ks = shift_ref.shape[0]
    qscale = float(Dh ** -0.5 * np.log2(np.e))

    x_cp = [pltpu.make_async_copy(x_hbm.at[0, pl.ds(c * _QB, _QB)],
                                  x_v.at[pl.ds(c * _QB, _QB)], sems.at[c])
            for c in range(NQ)]
    w_cp = pltpu.make_async_copy(w_hbm, w_v, sems.at[NQ])
    h_cp = pltpu.make_async_copy(h_hbm, h_v, sems.at[NQ + 1])
    bk_cp = pltpu.make_async_copy(bk_hbm.at[0], bk_v, sems.at[NQ + 2])
    bv_cp = pltpu.make_async_copy(bv_hbm.at[0], bv_v, sems.at[NQ + 3])
    wo_cp = pltpu.make_async_copy(wo_hbm, wo_v, sems.at[NQ + 4])
    w_cp.start()
    x_cp[0].start()
    w_cp.wait()
    for cp in x_cp[1:] + [h_cp, bk_cp, bv_cp, wo_cp]:
        cp.start()

    wt_v[0:D, :] = w_v[:, 0:D].T
    wt_v[D:2 * D, :] = w_v[:, 2 * D:3 * D].T

    row = lax.broadcasted_iota(jnp.int32, (_WIN, _QB), 0)
    lane = lax.broadcasted_iota(jnp.int32, (_QB // 2, 128), 1)

    def win_start(h):
        return (Dh * h) // 8 * 8

    def proj(c, carry):
        pltpu.make_async_copy(x_hbm.at[0, pl.ds(0, _QB)], x_v.at[pl.ds(0, _QB)],
                              sems.at[c]).wait()
        r0 = pl.multiple_of(c * _QB, _QB)
        xc = x_v[pl.ds(r0, _QB), :]
        kc = pltpu.bitcast(_dot(xc, w_v[:, D:2 * D]).astype(_BF16), jnp.uint32)
        qv = _dot(wt_v[...], xc, _NT)
        r1 = pl.multiple_of(c * (_QB // 2), _QB // 2)
        for h in range(_H):
            w = win_start(h)
            mine = (row >= Dh * h - w) & (row < Dh * (h + 1) - w)
            g, off = divmod(w, 128)
            kg = kc[:, g * 128:(g + 1) * 128]
            if off + _WIN > 128:
                kg = jnp.where(lane >= off, kg, kc[:, (g + 1) * 128:(g + 2) * 128])
            if off:
                kg = pltpu.roll(kg, 128 - off, 1)
            k_all[h, pl.ds(r1, _QB // 2), :] = kg
            q = jnp.where(mine, qv[w:w + _WIN] * qscale, 0.0)
            q = jnp.concatenate([q, jnp.zeros((32 - _WIN, _QB), _F32)], axis=0)
            q_all[h * NQ + c] = pltpu.bitcast(q.astype(_BF16), jnp.uint32)
            v = qv[D + w:D + w + _WIN].astype(_BF16).astype(_F32)
            v_all[h * NQ + c] = jnp.where(mine, v, 1.0)
        return carry

    lax.fori_loop(0, NQ, proj, 0)

    h_cp.wait()
    bk_cp.wait()
    bv_cp.wait()
    fwd = fwd_ref[...]
    sign = (1 - 2 * (lax.broadcasted_iota(jnp.int32, (_C, D), 0) & 1)).astype(_F32)
    g_prev = None
    for m in range(NC):
        g_cur = _dot(fwd, h_v[:, m * _C:(m + 1) * _C], _NT)
        if g_prev is None:
            hf_v[m] = g_cur
        else:
            hf_v[m, 0:_C] = g_cur[0:_C] - sign * g_prev[_C:]
            hf_v[m, _C:] = g_cur[_C:] + sign * g_prev[0:_C]
        g_prev = g_cur

    taps = shift_ref[...].astype(_F32)

    def ssm_fwd(j, tail):
        r0 = pl.multiple_of(j * _C, _C)
        kf = bk_v[pl.ds(r0, _C), :].astype(_F32)
        ext = jnp.concatenate([tail, kf], axis=0)
        acc = kf * taps[0:1]
        for t in range(1, ks):
            acc = acc + pltpu.roll(ext, t, 0)[8:] * taps[t:t + 1]
        kv = (acc * bv_v[pl.ds(r0, _C), :].astype(_F32)).astype(_BF16)
        kv_v[pl.ds(r0, _C), :] = kv
        xf_v[j] = _dot(fwd_ref[...], kv)
        return kf[_C - 8:]

    lax.fori_loop(0, NC, ssm_fwd, jnp.zeros((8, D), _F32), unroll=4)

    def ssm_mix(r):
        half = _C // 8
        imag = r >= half
        f0 = pl.multiple_of((r % half) * 8, 8)
        f1 = pl.multiple_of(f0 + _C, 8)
        own = pl.multiple_of(r * 8, 8)
        oth = pl.multiple_of(jnp.where(imag, f0, f1), 8)
        sgn = jnp.where(imag, 1.0, -1.0)
        for g in range(NG):
            cols = slice(g * 128, (g + 1) * 128)
            xa = [xf_v[j, pl.ds(own, 8), cols] for j in range(NC)]
            xb = [xf_v[j, pl.ds(oth, 8), cols] * sgn for j in range(NC)]
            hr = [hf_v[j, pl.ds(f0, 8), cols] for j in range(NC)]
            hi = [hf_v[j, pl.ds(f1, 8), cols] for j in range(NC)]
            for i in range(NC):
                acc = None
                for j in range(i + 1):
                    t = hr[i - j] * xa[j] + hi[i - j] * xb[j]
                    acc = t if acc is None else acc + t
                yf_v[i, pl.ds(own, 8), cols] = acc

    def ssm_mix_loop(r, carry):
        ssm_mix(r)
        return carry

    lax.fori_loop(0, 2 * _C // 8, ssm_mix_loop, 0)

    row8 = lax.broadcasted_iota(jnp.int32, (8, _QB), 0)

    def step(qk, pv, m):
        mx = acc = None
        for kc in range(NK):
            rows = slice(kc * _KC, (kc + 1) * _KC)
            if qk is not None:
                h, qb = qk
                lhs = pltpu.bitcast(
                    k_all[h, kc * _KC // 2:(kc + 1) * _KC // 2, :], _BF16)[:, :32]
                s = _dot(lhs, pltpu.bitcast(q_all[h * NQ + qb], _BF16))
                cm = jnp.max(s.reshape(_KC // 8, 8, _QB), axis=0)
                mx = cm if mx is None else jnp.maximum(mx, cm)
            if pv is not None:
                h, qb = pv
                p = jnp.exp2(s_buf[rows, :].reshape(_KC // 8, 8, _QB) - m[None])
                p = p.reshape(_KC, _QB).astype(_BF16)
                c, o = divmod(kc * _KC, _QB)
                r = _dot(v_all[h * NQ + c, :, o:o + _KC], p)
                acc = r if acc is None else acc + r
            if qk is not None:
                s_buf[rows, :] = s
        if pv is not None:
            h, qb = pv
            odd = h % 2
            w = Dh * h - 4 * odd
            if not isinstance(w, int):
                w = pl.multiple_of(w, 8)
            den = jnp.where(odd == 1, acc[0:1], acc[_WIN - 1:_WIN])
            o = acc * (1.0 / den)
            head = jnp.where(row8 < 4 * odd, ot_v[qb, pl.ds(w, 8), :], o[0:8])
            ot_v[qb, pl.ds(w, 8), :] = head
            ot_v[qb, pl.ds(w + 8, _WIN - 8), :] = o[8:]
        if qk is None:
            return None
        return jnp.broadcast_to(jnp.max(mx, axis=0, keepdims=True), (8, _QB))

    def head(h, m):
        for qb in range(NQ - 1):
            m = step((h, qb + 1), (h, qb), m)
        return step((h + 1, 0), (h, NQ - 1), m)

    m = step((0, 0), None, None)
    m = lax.fori_loop(0, _H - 1, head, m)
    for qb in range(NQ - 1):
        m = step((_H - 1, qb + 1), (_H - 1, qb), m)
    step(None, (_H - 1, NQ - 1), m)

    wo_cp.wait()
    gw = gw_ref[...].astype(_F32)
    dskip = d_ref[...].astype(_F32)

    def out_copy(c, r0):
        return pltpu.make_async_copy(out_v.at[pl.ds(r0, _QB)],
                                     out_hbm.at[0, pl.ds(r0, _QB)], osems.at[c])

    def finish(c, carry):
        a = _dot(ot_v[c].T.astype(_BF16), wo_v[...])
        for i in range(_QB // _C):
            r0 = pl.multiple_of(c * _QB + i * _C, _C)
            y = _dot(inv_ref[...], yf_v[c * (_QB // _C) + i].astype(_BF16))
            xf = x_v[pl.ds(r0, _C), :].astype(_F32)
            gate = jax.nn.sigmoid(jnp.sum(xf * gw, axis=-1, keepdims=True))
            b = xf * (y + kv_v[pl.ds(r0, _C), :].astype(_F32) * dskip)
            res = gate * a[i * _C:(i + 1) * _C] + (1.0 - gate) * b
            out_v[pl.ds(r0, _C), :] = res.astype(out_v.dtype)
        out_copy(c, pl.multiple_of(c * _QB, _QB)).start()
        return carry

    lax.fori_loop(0, NQ, finish, 0)
    for c in range(NQ):
        out_copy(c, c * _QB).wait()


@jax.jit
def pallas_gated_mix__mha_block__ssm_conv_h3__prompt_kernel(
    A_x: jax.Array,
    A_wqkv: jax.Array,
    A_wo: jax.Array,
    B_q: jax.Array,
    B_k: jax.Array,
    B_v: jax.Array,
    B_shift_k: jax.Array,
    B_ssm_k: jax.Array,
    B_ssm_D: jax.Array,
    gate_w: jax.Array,
):
    del B_q
    _, S, D = A_x.shape
    NQ, NC = S // _QB, S // _C
    fwd, inv = _dft_matrices()
    hbm = pl.BlockSpec(memory_space=pl.ANY)
    vmem = pl.BlockSpec(memory_space=pltpu.VMEM)
    return pl.pallas_call(
        _kernel,
        out_shape=jax.ShapeDtypeStruct(A_x.shape, A_x.dtype),
        in_specs=[hbm] * 6 + [vmem] * 5,
        out_specs=hbm,
        scratch_shapes=[
            pltpu.VMEM((S, D), _BF16),
            pltpu.VMEM((D, 3 * D), _BF16),
            pltpu.VMEM((2 * D, D), _BF16),
            pltpu.VMEM((D, D), _BF16),
            pltpu.VMEM((S, D), _BF16),
            pltpu.VMEM((S, D), _BF16),
            pltpu.VMEM((D, S), _BF16),
            pltpu.VMEM((_H, S // 2, 128), jnp.uint32),
            pltpu.VMEM((_H * NQ, 16, _QB), jnp.uint32),
            pltpu.VMEM((_H * NQ, _WIN, _QB), _F32),
            pltpu.VMEM((S, _QB), _F32),
            pltpu.VMEM((NQ, D, _QB), _F32),
            pltpu.VMEM((S, D), _BF16),
            pltpu.VMEM((NC, 2 * _C, D), _F32),
            pltpu.VMEM((NC, 2 * _C, D), _F32),
            pltpu.VMEM((NC, 2 * _C, D), _F32),
            pltpu.VMEM((S, D), A_x.dtype),
            pltpu.SemaphoreType.DMA((NQ + 5,)),
            pltpu.SemaphoreType.DMA((NQ,)),
        ],
        compiler_params=pltpu.CompilerParams(vmem_limit_bytes=110 * 1024 * 1024),
    )(A_x, A_wqkv, A_wo, B_k, B_v, B_ssm_k,
      B_shift_k.T, B_ssm_D.reshape(1, D), gate_w.reshape(1, D),
      fwd.astype(_BF16), inv.astype(_BF16))
```

```python
import numpy as np
import jax
import jax.numpy as jnp
from jax import lax
import jax.experimental.pallas as pl
import jax.experimental.pallas.tpu as pltpu

_H = 32
_QB = 512
_KC = 128
_WIN = 24
_KWIN = 32
_C = 128
_PAT = ((3, 9), (1, 6, 11), (3, 10), (1, 5, 11))
_PIECES = (14, 14, 14, 14, 14, 12, 14, 14, 14, 12, 14, 14, 14, 12, 14, 12)
_X_CHUNKS = (0, 2, 6, 16)
_SSM_CHUNKS = (0, 8, 12, 16)
_FIN = 8
_DEN_RANGE = (2.0 ** -20, 2.0 ** 40)

_NN = (((1,), (0,)), ((), ()))
_NT = (((1,), (1,)), ((), ()))
_F32 = jnp.float32
_BF16 = jnp.bfloat16
_U32 = jnp.uint32


def _dft_matrices():
    even = np.arange(0, _C, 2)
    freq = np.concatenate([even, _C - 1 - even])
    ang = (np.pi * (freq + 0.5) / _C)[:, None] * np.arange(_C)[None, :]
    fwd = np.concatenate([np.cos(ang), -np.sin(ang)], axis=0)
    ang = ang[:_C // 2].T
    inv = np.concatenate([np.cos(ang), -np.sin(ang)], axis=1) / _C
    split = np.concatenate([fwd[:, 0::2], fwd[:, 1::2]], axis=1)
    return np.concatenate([fwd, inv[0::2], inv[1::2], split], axis=0).astype(np.float32)


def _key_plan(nk):
    plan, counts, bounds = [], {"m": 0, "v": 0}, [0]
    for k in range(nk):
        pos = _PAT[k % len(_PAT)]
        kinds = []
        for i in range(_KC // 8 - len(pos) + 1):
            kinds += ["v"] * pos.count(i) + ["m"]
        tile = []
        for kind in kinds[:-1]:
            tile.append((kind, counts[kind]))
            counts[kind] += 1
        plan.append(tile)
        bounds.append(bounds[-1] + _PIECES[k])
        assert bounds[-1] >= counts["m"]
    assert bounds[-1] == counts["m"]
    return plan, bounds, counts["m"], counts["v"]


def _dot(a, b, dims=_NN):
    return lax.dot_general(a, b, dims, preferred_element_type=_F32)


def _aligned(i, n):
    return i if isinstance(i, int) else pl.multiple_of(i, n)


def _tile(g, n=1):
    return slice(g * 128, (g + n) * 128)


def _kernel(x_hbm, w_hbm, wo_hbm, bk_hbm, bv_hbm, h_hbm, shift_hbm, d_hbm, gw_hbm, dft_hbm,
            out_hbm,
            xp_v, x_v, w_v, wo_v, bk_v, bv_v, h_v,
            km_v, kp_v, kt_v, kph_v, kb_a, kb_b, q_v, qb_v, v_v, p_v, acc_v,
            den_v, rcp_v, gt_v, xg_v, o_v, xf_v, hf_v, yw_v, pj_v, y_v, out_v,
            dft_v, shift_v, d_v, gw_v, sems, osem):
    S, D = x_v.shape
    Dh = D // _H
    NQ, NK, NC, NG = S // _QB, S // _KC, S // _C, D // 128
    NT = _QB // 128
    FG = _C // 8
    WT0 = (NC + 1) * 2 * FG
    plan, bounds, NM, NV = _key_plan(NK)
    kb_v = (kb_a, kb_b)
    row = lax.broadcasted_iota(jnp.int32, (8, 128), 0)

    used = []

    def copy(src, dst):
        used.append(None)
        return pltpu.make_async_copy(src, dst, sems.at[len(used) - 1])

    def copy_rows(src, dst, lo, hi):
        return copy(src.at[0, pl.ds(lo, hi - lo)], dst.at[pl.ds(lo, hi - lo)])

    def arrive(copies):
        for cp in copies:
            cp.wait()

    x_cp = {lo: copy_rows(x_hbm, x_v, lo * _KC, hi * _KC)
            for lo, hi in zip(_X_CHUNKS[:-1], _X_CHUNKS[1:])}
    w_cp = [copy(w_hbm.at[:, pl.ds(i * D, D)], w_v.at[i]) for i in range(3)]
    ssm_cp = {lo: [copy(h_hbm.at[:, pl.ds(lo * _C, (hi - lo) * _C)],
                        h_v.at[:, pl.ds(lo * _C, (hi - lo) * _C)]),
                   copy_rows(bk_hbm, bk_v, lo * _C, hi * _C),
                   copy_rows(bv_hbm, bv_v, lo * _C, hi * _C)]
              for lo, hi in zip(_SSM_CHUNKS[:-1], _SSM_CHUNKS[1:])}
    ssm_cp[0] += [copy(dft_hbm, dft_v), copy(shift_hbm, shift_v), copy(d_hbm, d_v)]
    gw_cp = copy(gw_hbm, gw_v)
    wo_cp = copy(wo_hbm, wo_v)
    for cp in ([gw_cp, w_cp[1]] + list(x_cp.values()) + sum(ssm_cp.values(), [])
               + [w_cp[0], w_cp[2]]):
        cp.start()
    yw_v[0:2 * FG] = jnp.zeros((2 * FG, 8, D), _F32)
    arrive([gw_cp, w_cp[1], x_cp[0]])

    def head_cols(a, h):
        w = (Dh * h) // 16 * 16
        g, off = divmod(w, 128)
        t = a[:, _tile(g)]
        lane = lax.broadcasted_iota(jnp.int32, t.shape, 1)
        if off + _KWIN > 128:
            t = jnp.where(lane >= off, t, a[:, _tile(g + 1)])
        if off:
            t = pltpu.roll(t, 128 - off, 1)
        return jnp.where((lane >= Dh * h - w) & (lane < Dh * (h + 1) - w), t, jnp.zeros_like(t))

    half_gw = 0.5 * gw_v[...].astype(_F32).reshape(1, D)
    held = []
    for kc in range(NK):
        xc = x_v[kc * _KC:(kc + 1) * _KC, :]
        xp_v[kc * _KC // 2:(kc + 1) * _KC // 2, :] = pltpu.bitcast(xc, _U32)
        xf = xc.astype(_F32)
        tilt = 0.5 * jnp.tanh(jnp.sum(xf * half_gw, axis=-1, keepdims=True))
        xg_v[kc * _KC:(kc + 1) * _KC, :] = xf * (0.5 - tilt)
        gt_v[kc] = 0.5 + jnp.broadcast_to(tilt, (_KC, 128)).T[:8]
        kf = _dot(xc, w_v[1]) * float(Dh ** -0.5 * np.log2(np.e))
        mine = []
        for j, (kind, idx) in zip(range(_KC // 8 - 1, -1, -1), plan[kc]):
            (mine if kind == "v" else held).append((idx, kf[8 * j:8 * j + 8]))
        n = len(held) // 2 * 2
        km = jnp.concatenate([t for _, t in held[:n]], axis=0)
        km = pltpu.bitcast(km.astype(_BF16), _U32)
        for h in range(_H):
            if h == 12 and kc + 1 in x_cp:
                arrive([x_cp[kc + 1]])
            if h == 12 and kc + 1 == NK:
                arrive(ssm_cp[0])
            lo = 4 * (h * NM + held[0][0])
            km_v[lo:lo + 4 * n, :] = head_cols(km, h)
        for idx, t in mine:
            kp_v[8 * idx:8 * idx + 8, :] = t
        held = held[n:]

    for c in range(kt_v.shape[0]):
        n = min(128, 8 * NV - 128 * c)
        t = kp_v[128 * c:128 * c + n, :].astype(_BF16).astype(_F32)
        kt_v[c] = jnp.concatenate(
            [pltpu.roll(t, D - r, 1) if r else t for r in range(128 // n)], axis=0).T

    def spread_keys(h, slot, never=None):
        last = None
        for c in range(kt_v.shape[0] - 1, -1, -1):
            n = min(128, 8 * NV - 128 * c)
            for d in range(0, Dh, 128 // n):
                r = jnp.broadcast_to(kt_v[c, pl.ds(h * Dh + d, 1), :], (8, 128))
                if never is not None and last is not None:
                    r = jnp.where(never, last[:8], r)
                last = jnp.concatenate([r] * 16, axis=0).T
                for i in range(128 // n):
                    kb_v[slot][0, 16 * c:16 * c + n // 8, d + i] = (
                        last[i * n:(i + 1) * n].reshape(n // 8, 8, 128))

    spread_keys(0, 0)

    taps = shift_v[...].astype(_F32)
    dskip = d_v[...].astype(_F32).reshape(1, D)
    ks = taps.shape[0]
    per = _QB // _C

    def row_of_pair(words, odd):
        return pltpu.bitcast(words & _U32(0xFFFF0000) if odd else words << 16, _F32)

    def shifted_kv(c, cols):
        words = pltpu.bitcast(bk_v[max(c * _QB - 16, 0):(c + 1) * _QB, cols], _U32)
        if c == 0:
            words = jnp.concatenate([jnp.zeros((8, 128), _U32), words], axis=0)
        back = [words[8:]] + [pltpu.roll(words, t, 0)[8:] for t in range(1, ks // 2 + 1)]
        vals = pltpu.bitcast(bv_v[c * _QB:(c + 1) * _QB, cols], _U32)
        kv = []
        for par in range(2):
            acc = None
            for t in range(ks):
                term = row_of_pair(back[(t + 1 - par) // 2], (par - t) % 2) * taps[t:t + 1, cols]
                acc = term if acc is None else acc + term
            kv.append(acc * row_of_pair(vals, par))
        n = _C // 2
        return jnp.concatenate(
            [jnp.concatenate([kv[0][i * n:(i + 1) * n], kv[1][i * n:(i + 1) * n]], axis=0)
             for i in range(per)], axis=1)

    for c in range(NQ):
        if c and c * per in ssm_cp:
            arrive(ssm_cp[c * per])
        for g in range(NG):
            if (c, g) == (NQ - 1, NG - 2):
                arrive([w_cp[0], w_cp[2]])
                for i in range(2):
                    yw_v[WT0 + i * D // 16:WT0 + (i + 1) * D // 16] = (
                        pltpu.bitcast(w_v[2 * i].T, _F32).reshape(D // 16, 8, D))
            chunks = range(c * per, (c + 1) * per)
            taps_t = jnp.concatenate([h_v[_tile(g), _tile(j)] for j in chunks], axis=0)
            res = _dot(dft_v[0:2 * _C, :], taps_t, _NT)
            for i, j in enumerate(chunks):
                t = res[:, _tile(i)]
                if j == 0:
                    t = jnp.concatenate([t[:_C] + dskip[:, _tile(g)], t[_C:]], axis=0)
                hf_v[j, :, :, :, _tile(g)] = t.reshape(2, FG, 8, 128)
            res = _dot(dft_v[3 * _C:5 * _C, :], shifted_kv(c, _tile(g)))
            for i, j in enumerate(chunks):
                xf_v[j, :, :, :, _tile(g)] = res[:, _tile(i)].reshape(2, FG, 8, 128)

    pins = []

    def chunk_conv(first, fg, g, zeros):
        half = NC // 2
        order = [k for i in range(half // 2) for k in (i, half - 1 - i)]

        def load(ref, imag, z):
            return ref[:, imag, (first + zeros[z]) + fg, :, _tile(g)]

        def pin(val):
            pins.append(None)
            yw_v[zeros[0] + (WT0 + D // 8 + len(pins) % 3), :, _tile(g)] = val

        def tri(a, b, i):
            acc = a[i] * b[0]
            for j in range(1, i + 1):
                acc = acc + a[i - j] * b[j]
            return acc

        def conv(a, b, emit):
            a, b = ([t[j] for j in range(NC)] for t in (a, b))
            part = {}
            for par in range(2):
                for i in order:
                    part[par, i] = tri(a[par::2], b[par::2], i)
                    pin(part[par, i])
                    yield 2 * i + 2
            sa, sb = ([t[2 * i] + t[2 * i + 1] for i in range(half)] for t in (a, b))
            for i in order:
                emit(2 * i, part[0, i] + part[1, i - 1] if i else part[0, i])
                emit(2 * i + 1, tri(sa, sb, i) - part[0, i] - part[1, i])
                yield 2 * i + 7

        common = {}

        def keep(i, t):
            common[i] = t
            pin(t)

        def real(i, t):
            yw_v[first + ((2 * i + 2) * FG + fg), :, _tile(g)] = common[i] - t

        def imag(i, t):
            yw_v[first + ((2 * i + 3) * FG + fg), :, _tile(g)] = common[i] + t

        yield from conv(load(xf_v, 0, 0) + load(xf_v, 1, 0), load(hf_v, 0, 0), keep)
        yield from conv(load(hf_v, 0, 1) + load(hf_v, 1, 1), load(xf_v, 1, 1), real)
        yield from conv(load(hf_v, 1, 2) - load(hf_v, 0, 2), load(xf_v, 0, 2), imag)

    def qv_proj(c, carry):
        n = FG // NQ
        zeros = [lax.shift_right_logical(c, 8 + i) for i in range(3)]
        work = (ops for i in range(n) for g in range(NG) for ops in chunk_conv(c * n, i, g, zeros))
        slots = 2 * D // 16
        per_slot = n * NG * 768 / (slots * NG + 3)
        budget = [0.0]

        def weights(cols):
            out = []
            for i in range(slots):
                while budget[0] > 0:
                    budget[0] -= next(work, budget[0])
                budget[0] += per_slot
                out.append(yw_v[WT0 + i, :, cols])
            return pltpu.bitcast(jnp.concatenate(out, axis=0), _BF16)

        def x_rows(j, m, cols):
            r0 = pl.multiple_of(c * (_QB // 2) + j * 64, 64)
            return pltpu.bitcast(xp_v[pl.ds(r0, m * 64), cols], _BF16)

        pj_v[...] = _dot(weights(_tile(NG - 1)), x_rows(0, NT, _tile(NG - 1)), _NT)
        for j in range(NT):
            r = _dot(weights(_tile(0, NG - 1)), x_rows(j, 1, _tile(0, NG - 1)), _NT)
            r = r + pj_v[:, _tile(j)]
            q_v[pl.ds(c * (D // 8), D // 8), :, _tile(j)] = r[:D].reshape(D // 8, 8, 128)
            qb_v[pl.ds(pl.multiple_of(c * (D // 2), 8), D // 2), _tile(j)] = (
                pltpu.bitcast(r[:D].astype(_BF16), _U32))
            for h in range(0, _H, 2):
                t = r[D + h * Dh:D + (h + 2) * Dh]
                v_v[h * NQ + c, :, _tile(j)] = jnp.concatenate(
                    [t[:16], jnp.where(row < 4, t[16:24], 1.0)], axis=0)
                v_v[(h + 1) * NQ + c, :, _tile(j)] = jnp.concatenate(
                    [jnp.where(row < 4, 1.0, t[16:24]), t[24:]], axis=0)
        for _ in work:
            pass
        return carry

    lax.fori_loop(0, NQ, qv_proj, 0)

    def write_head(h, odd, qb, acc):
        den = acc[0:1] if odd else acc[_WIN - 1:_WIN]
        for j in range(NT):
            o_v[qb * NT + j, pl.ds(_aligned(h * _WIN, 8), _WIN), :] = acc[:, _tile(j)]
            den_v[qb * NT + j, pl.ds(h, 1), :] = den[:, _tile(j)]

    def q_window(h, qb):
        w = _aligned(qb * (D // 2) + ((Dh * h) >> 4) * 8, 8)
        return pltpu.bitcast(qb_v[pl.ds(w, _KWIN // 2), :], _BF16)

    def mxu_scores(h, qb, lo, n):
        keys = km_v[pl.ds(_aligned(4 * NM * h + 4 * lo, 8), 4 * n), :]
        return _dot(pltpu.bitcast(keys, _BF16)[:, :_KWIN], q_window(h, qb))

    def mxu_probs(h, qb, kc):
        lo, n = bounds[kc], bounds[kc + 1] - bounds[kc]
        p = jnp.exp2(mxu_scores(h, qb, lo, n))
        return {("m", lo + i): p[8 * i:8 * i + 8] for i in range(n)}

    def head_pair(i, carry):
        never = row > i + 8
        never_wide = lax.broadcasted_iota(jnp.int32, (8, _QB), 0) > i + 8
        zero = lax.shift_right_logical(i, 8)
        probs = {("m", k): p_v[8 * k:8 * k + 8, :] for k in range(bounds[1])}
        s = None
        for odd in range(2):
            h = 2 * i + odd
            nxt = jnp.minimum(h + 1, _H - 2) if odd else h + 1
            spread_keys(nxt, 1 - odd, never)
            rows = [divmod(d + 4 * odd, 8) for d in range(Dh)]
            for qb in range(NQ):
                for kc in range(NK):
                    if kc + 1 < NK:
                        ahead = mxu_probs(h, qb, kc + 1)
                    elif qb + 1 < NQ:
                        ahead = mxu_probs(h, qb + 1, 0)
                    else:
                        ahead = mxu_probs(nxt, 0, 0)
                    for kind, idx in plan[kc]:
                        if kind == "m":
                            continue
                        zero = lax.shift_right_logical(zero, 1)
                        base = qb * (D // 8) + ((Dh * h) >> 3) + zero
                        first = [base + hi for hi in range(_WIN // 8)]
                        keys = kb_v[odd][zero, idx].reshape(Dh * 8, 128)
                        for d, (hi, lo) in enumerate(rows):
                            key = keys[8 * d:8 * d + 8]
                            term = jnp.concatenate(
                                [key * q_v[first[hi], lo:lo + 1, _tile(j)] for j in range(NT)], axis=1)
                            if d:
                                s = s + term
                            else:
                                s = term if s is None else jnp.where(never_wide, s, term)
                        probs[kind, idx] = jnp.exp2(s)
                    tile = jnp.concatenate([probs.pop(key) for key in plan[kc][::-1]], axis=0)
                    r = _dot(v_v[h * NQ + kc // NT, :, _tile(kc % NT)], tile)
                    probs.update(ahead)
                    if kc == 0:
                        acc_v[...] = r
                    else:
                        acc = r + (acc_v[...] if kc == 1 else acc)
                write_head(h, odd, qb, acc)
        for k in range(bounds[1]):
            p_v[8 * k:8 * k + 8, :] = probs["m", k]
        return carry

    wo_cp.start()
    for (_, k), p in mxu_probs(0, 0, 0).items():
        p_v[8 * k:8 * k + 8, :] = p
    lax.fori_loop(0, _H // 2, head_pair, 0)

    den = den_v[...]
    safe = (den >= _DEN_RANGE[0]) & (den <= _DEN_RANGE[1])
    unsafe = jnp.max(jnp.max(jnp.where(safe, 0.0, 1.0), axis=0)).astype(jnp.int32)

    @pl.when(unsafe > 0)
    def _redo_with_true_row_max():
        def regroup(i, carry):
            r = pl.ds(pl.multiple_of(i * 8, 8), 8)
            for h in range(_H):
                kph_v[h, r, :] = head_cols(kp_v[r, :], h)
            return carry

        lax.fori_loop(0, NV, regroup, 0)

        def unit(u, carry):
            h, qb = u // NQ, u % NQ

            def scores(c):
                keys = kph_v[h, pl.ds(pl.multiple_of(c * (8 * NV // NQ), 8), 8 * NV // NQ), :]
                return {"m": mxu_scores(h, qb, c * (NM // NQ), NM // NQ),
                        "v": _dot(keys[:, :_KWIN], q_window(h, qb))}

            def running_max(c, m):
                for s in scores(c).values():
                    m = jnp.maximum(m, jnp.max(s, axis=0, keepdims=True))
                return m

            m = lax.fori_loop(0, NQ, running_max, jnp.full((1, _QB), -jnp.inf, _F32))

            def accumulate(c, acc):
                s = scores(c)
                p = [jnp.exp2(s[kind][8 * i:8 * i + 8] - m)
                     for kc in range(NK // NQ) for kind, i in plan[kc][::-1]]
                return acc + _dot(v_v[h * NQ + c], jnp.concatenate(p, axis=0))

            acc = lax.fori_loop(0, NQ, accumulate, jnp.zeros((_WIN, _QB), _F32))
            for odd in range(2):
                pl.when(h % 2 == odd)(lambda: write_head(h, odd, qb, acc))
            return carry

        lax.fori_loop(0, _H * NQ, unit, 0)

    wo_cp.wait()

    def finish(c, carry):
        for i in range(_FIN):
            j = c * _FIN + i
            out_rows = pl.ds(pl.multiple_of(j * _C, _C), _C)
            rcp_v[i] = jnp.concatenate([gt_v[j]] * (_H // 8), axis=0) / den_v[j]
            heads = []
            for h in range(0, _H, 2):
                e, f = (o_v[j, (h + u) * _WIN:(h + u + 1) * _WIN, :]
                        * jnp.broadcast_to(rcp_v[i, h + u:h + u + 1, :], (_WIN, 128))
                        for u in range(2))
                heads += [e[:16], jnp.where(row < 4, e[16:], f[:8]), f[8:]]
            o = jnp.concatenate(heads, axis=0).T.astype(_BF16)
            base = 2 * j * FG + lax.shift_right_logical(c, 8 + i % 2)
            res = []
            for g in range(NG):
                z = yw_v[pl.ds(base, 4 * FG), :, _tile(g)].reshape(8, _C // 2, 128)
                ar, br, ai, bi = z[4] - z[2], z[5] + z[3], z[6] + z[0], z[7] - z[1]
                for par in range(2):
                    lo = 2 * _C + par * _C // 2
                    y_v[i % 4 * NG + g, pl.ds(par, _C // 2, stride=2), :] = _dot(
                        dft_v[lo:lo + _C // 2, :],
                        jnp.concatenate((ar - br, ai + bi) if par else (ar + br, ai - bi), axis=0))
                res.append(_dot(o, wo_v[:, _tile(g)])
                           + xg_v[out_rows, _tile(g)] * y_v[i % 4 * NG + g])
            out_v[out_rows, :] = jnp.concatenate(res, axis=1).astype(out_v.dtype)
            pltpu.make_async_copy(out_v.at[out_rows], out_hbm.at[0, out_rows], osem).start()
        return carry

    lax.fori_loop(0, NC // _FIN, finish, 0)
    pltpu.make_async_copy(out_v, out_hbm.at[0], osem).wait()


@jax.jit
def pallas_gated_mix__mha_block__ssm_conv_h3__prompt_kernel(
    A_x: jax.Array,
    A_wqkv: jax.Array,
    A_wo: jax.Array,
    B_q: jax.Array,
    B_k: jax.Array,
    B_v: jax.Array,
    B_shift_k: jax.Array,
    B_ssm_k: jax.Array,
    B_ssm_D: jax.Array,
    gate_w: jax.Array,
):
    del B_q
    _, S, D = A_x.shape
    NQ, NC = S // _QB, S // _C
    _, _, NM, NV = _key_plan(S // _KC)
    hbm = pl.BlockSpec(memory_space=pl.ANY)
    vmem = pltpu.VMEM
    return pl.pallas_call(
        _kernel,
        out_shape=jax.ShapeDtypeStruct(A_x.shape, A_x.dtype),
        in_specs=[hbm] * 10,
        out_specs=hbm,
        scratch_shapes=[
            vmem((S // 2, D), _U32),
            vmem((S, D), _BF16),
            vmem((3, D, D), _BF16),
            vmem((D, D), _BF16),
            vmem((S, D), _BF16),
            vmem((S, D), _BF16),
            vmem((D, S), _BF16),
            vmem((_H * 4 * NM, 128), _U32),
            vmem((8 * NV, D), _F32),
            vmem((-(-8 * NV // 128), D, 128), _F32),
            vmem((_H, 8 * NV, 128), _F32),
            vmem((1, NV, D // _H, 8, 128), _F32),
            vmem((1, NV, D // _H, 8, 128), _F32),
            vmem((NQ * D // 8, 8, _QB), _F32),
            vmem((NQ * D // 2, _QB), _U32),
            vmem((_H * NQ, _WIN, _QB), _F32),
            vmem((_KC, _QB), _F32),
            vmem((_WIN, _QB), _F32),
            vmem((S // 128, _H, 128), _F32),
            vmem((_FIN, _H, 128), _F32),
            vmem((S // 128, 8, 128), _F32),
            vmem((S, D), _F32),
            vmem((S // 128, _H * _WIN, 128), _F32),
            vmem((NC, 2, _C // 8, 8, D), _F32),
            vmem((NC, 2, _C // 8, 8, D), _F32),
            vmem(((S + _C) // 4 + D // 8 + 4, 8, D), _F32),
            vmem((2 * D, _QB), _F32),
            vmem((4 * D // 128, _C, 128), _F32),
            vmem((S, D), A_x.dtype),
            vmem((5 * _C, _C), _BF16),
            vmem(B_shift_k.shape[::-1], _BF16),
            vmem((D,), _BF16),
            vmem((D,), _BF16),
            pltpu.SemaphoreType.DMA((len(_X_CHUNKS) + 3 * len(_SSM_CHUNKS) + 4,)),
            pltpu.SemaphoreType.DMA(()),
        ],
        compiler_params=pltpu.CompilerParams(vmem_limit_bytes=120 * 1024 * 1024),
    )(A_x, A_wqkv, A_wo, B_k, B_v, B_ssm_k, B_shift_k.T, B_ssm_D, gate_w,
      _dft_matrices().astype(_BF16))
```

```python
import numpy as np
import jax
import jax.numpy as jnp
from jax import lax
import jax.experimental.pallas as pl
import jax.experimental.pallas.tpu as pltpu

_H = 32
_QB = 512
_KC = 128
_WIN = 24
_KWIN = 32
_C = 128
_PAT = ((3, 9), (2, 6, 12), (4, 10), (1, 5, 11))
_PIECES = (16, 14, 14, 12, 14, 14, 14, 12, 14, 14, 14, 12, 14, 12, 14, 12)
_X_CHUNKS = (0, 2, 6, 16)
_SSM_CHUNKS = (0, 8, 12, 16)
_FIN = 8
_DEN_RANGE = (2.0 ** -30, 2.0 ** 50)

_NN = (((1,), (0,)), ((), ()))
_NT = (((1,), (1,)), ((), ()))
_F32 = jnp.float32
_BF16 = jnp.bfloat16
_U32 = jnp.uint32


def _dft_matrices():
    even = np.arange(0, _C, 2)
    freq = np.concatenate([even, _C - 1 - even])
    ang = (np.pi * (freq + 0.5) / _C)[:, None] * np.arange(_C)[None, :]
    fwd = np.concatenate([np.cos(ang), -np.sin(ang)], axis=0)
    ang = ang[:_C // 2].T
    inv = np.concatenate([np.cos(ang), -np.sin(ang)], axis=1) / _C
    split = np.concatenate([fwd[:, 0::2], fwd[:, 1::2]], axis=1)
    return np.concatenate([fwd, inv[0::2], inv[1::2], split], axis=0).astype(np.float32)


def _key_plan(nk):
    plan, counts, bounds = [], {"m": 0, "v": 0}, [0]
    for k in range(nk):
        pos = _PAT[k % len(_PAT)]
        kinds = []
        for i in range(_KC // 8 - len(pos) + 1):
            kinds += ["v"] * pos.count(i) + ["m"]
        tile = []
        for kind in kinds[:-1]:
            tile.append((kind, counts[kind]))
            counts[kind] += 1
        plan.append(tile)
        bounds.append(bounds[-1] + _PIECES[k])
        assert bounds[-1] >= counts["m"]
    assert bounds[-1] == counts["m"]
    return plan, bounds, counts["m"], counts["v"]


def _dot(a, b, dims=_NN):
    return lax.dot_general(a, b, dims, preferred_element_type=_F32)


def _aligned(i, n):
    return i if isinstance(i, int) else pl.multiple_of(i, n)


def _tile(g, n=1):
    return slice(g * 128, (g + n) * 128)


def _kernel(x_hbm, w_hbm, wo_hbm, bk_hbm, bv_hbm, h_hbm, shift_hbm, d_hbm, gw_hbm, dft_hbm,
            out_hbm,
            xp_v, x_v, w_v, wo_v, bk_v, bv_v, h_v,
            km_v, kp_v, kt_v, kph_v, kb_a, kb_b, q_v, qb_v, v_v, p_v, acc_v,
            den_v, rcp_v, gt_v, xg_v, o_v, xf_v, hf_v, yw_v, pj_v, y_v, out_v,
            dft_v, shift_v, d_v, gw_v, sems, osem):
    S, D = x_v.shape
    Dh = D // _H
    NQ, NK, NC, NG = S // _QB, S // _KC, S // _C, D // 128
    NT = _QB // 128
    FG = _C // 8
    WT0 = (NC + 1) * 2 * FG
    plan, bounds, NM, NV = _key_plan(NK)
    kb_v = (kb_a, kb_b)
    row = lax.broadcasted_iota(jnp.int32, (8, 128), 0)

    used = []

    def copy(src, dst):
        used.append(None)
        return pltpu.make_async_copy(src, dst, sems.at[len(used) - 1])

    def copy_rows(src, dst, lo, hi):
        return copy(src.at[0, pl.ds(lo, hi - lo)], dst.at[pl.ds(lo, hi - lo)])

    def arrive(copies):
        for cp in copies:
            cp.wait()

    x_cp = {lo: copy_rows(x_hbm, x_v, lo * _KC, hi * _KC)
            for lo, hi in zip(_X_CHUNKS[:-1], _X_CHUNKS[1:])}
    w_cp = [copy(w_hbm.at[:, pl.ds(i * D, D)], w_v.at[i]) for i in range(3)]
    ssm_cp = {lo: [copy(h_hbm.at[:, pl.ds(lo * _C, (hi - lo) * _C)],
                        h_v.at[:, pl.ds(lo * _C, (hi - lo) * _C)]),
                   copy_rows(bk_hbm, bk_v, lo * _C, hi * _C),
                   copy_rows(bv_hbm, bv_v, lo * _C, hi * _C)]
              for lo, hi in zip(_SSM_CHUNKS[:-1], _SSM_CHUNKS[1:])}
    ssm_cp[0] += [copy(dft_hbm, dft_v), copy(shift_hbm, shift_v), copy(d_hbm, d_v)]
    gw_cp = copy(gw_hbm, gw_v)
    wo_cp = copy(wo_hbm, wo_v)
    for cp in ([gw_cp, w_cp[1]] + list(x_cp.values()) + sum(ssm_cp.values(), [])
               + [w_cp[0], w_cp[2]]):
        cp.start()
    yw_v[0:2 * FG] = jnp.zeros((2 * FG, 8, D), _F32)
    arrive([gw_cp, w_cp[1], x_cp[0]])

    def head_cols(a, h):
        w = (Dh * h) // 16 * 16
        g, off = divmod(w, 128)
        t = a[:, _tile(g)]
        lane = lax.broadcasted_iota(jnp.int32, t.shape, 1)
        if off + _KWIN > 128:
            t = jnp.where(lane >= off, t, a[:, _tile(g + 1)])
        if off:
            t = pltpu.roll(t, 128 - off, 1)
        return jnp.where((lane >= Dh * h - w) & (lane < Dh * (h + 1) - w), t, jnp.zeros_like(t))

    half_gw = 0.5 * gw_v[...].astype(_F32).reshape(1, D)
    held = []
    for kc in range(NK):
        xc = x_v[kc * _KC:(kc + 1) * _KC, :]
        xp_v[kc * _KC // 2:(kc + 1) * _KC // 2, :] = pltpu.bitcast(xc, _U32)
        xf = xc.astype(_F32)
        tilt = 0.5 * jnp.tanh(jnp.sum(xf * half_gw, axis=-1, keepdims=True))
        xg_v[kc * _KC:(kc + 1) * _KC, :] = xf * (0.5 - tilt)
        gt_v[kc] = 0.5 + jnp.broadcast_to(tilt, (_KC, 128)).T[:8]
        kf = _dot(xc, w_v[1]) * float(Dh ** -0.5 * np.log2(np.e))
        mine = []
        for j, (kind, idx) in zip(range(_KC // 8 - 1, -1, -1), plan[kc]):
            (mine if kind == "v" else held).append((idx, kf[8 * j:8 * j + 8]))
        n = len(held) // 2 * 2
        km = jnp.concatenate([t for _, t in held[:n]], axis=0)
        km = pltpu.bitcast(km.astype(_BF16), _U32)
        for h in range(_H):
            if h == 12 and kc + 1 in x_cp:
                arrive([x_cp[kc + 1]])
            if h == 12 and kc + 1 == NK:
                arrive(ssm_cp[0])
            lo = 4 * (h * NM + held[0][0])
            km_v[lo:lo + 4 * n, :] = head_cols(km, h)
        for idx, t in mine:
            kp_v[8 * idx:8 * idx + 8, :] = t
        held = held[n:]

    for c in range(kt_v.shape[0]):
        n = min(128, 8 * NV - 128 * c)
        t = kp_v[128 * c:128 * c + n, :].astype(_BF16).astype(_F32)
        kt_v[c] = jnp.concatenate(
            [pltpu.roll(t, D - r, 1) if r else t for r in range(128 // n)], axis=0).T

    def spread_keys(h, slot, never=None):
        last = None
        for c in range(kt_v.shape[0] - 1, -1, -1):
            n = min(128, 8 * NV - 128 * c)
            for d in range(0, Dh, 128 // n):
                r = jnp.broadcast_to(kt_v[c, pl.ds(h * Dh + d, 1), :], (8, 128))
                if never is not None and last is not None:
                    r = jnp.where(never, last[:8], r)
                last = jnp.concatenate([r] * 16, axis=0).T
                for i in range(128 // n):
                    kb_v[slot][0, 16 * c:16 * c + n // 8, d + i] = (
                        last[i * n:(i + 1) * n].reshape(n // 8, 8, 128))

    spread_keys(0, 0)

    taps = shift_v[...].astype(_F32)
    dskip = d_v[...].astype(_F32).reshape(1, D)
    ks = taps.shape[0]
    per = _QB // _C

    def row_of_pair(words, odd):
        return pltpu.bitcast(words & _U32(0xFFFF0000) if odd else words << 16, _F32)

    def shifted_kv(c, cols):
        words = pltpu.bitcast(bk_v[max(c * _QB - 16, 0):(c + 1) * _QB, cols], _U32)
        if c == 0:
            words = jnp.concatenate([jnp.zeros((8, 128), _U32), words], axis=0)
        back = [words[8:]] + [pltpu.roll(words, t, 0)[8:] for t in range(1, ks // 2 + 1)]
        vals = pltpu.bitcast(bv_v[c * _QB:(c + 1) * _QB, cols], _U32)
        kv = []
        for par in range(2):
            acc = None
            for t in range(ks):
                term = row_of_pair(back[(t + 1 - par) // 2], (par - t) % 2) * taps[t:t + 1, cols]
                acc = term if acc is None else acc + term
            kv.append(acc * row_of_pair(vals, par))
        n = _C // 2
        return jnp.concatenate(
            [jnp.concatenate([kv[0][i * n:(i + 1) * n], kv[1][i * n:(i + 1) * n]], axis=0)
             for i in range(per)], axis=1)

    for c in range(NQ):
        if c and c * per in ssm_cp:
            arrive(ssm_cp[c * per])
        for g in range(NG):
            if (c, g) == (NQ - 1, NG - 2):
                arrive([w_cp[0], w_cp[2]])
                for i in range(2):
                    yw_v[WT0 + i * D // 16:WT0 + (i + 1) * D // 16] = (
                        pltpu.bitcast(w_v[2 * i].T, _F32).reshape(D // 16, 8, D))
            chunks = range(c * per, (c + 1) * per)
            taps_t = jnp.concatenate([h_v[_tile(g), _tile(j)] for j in chunks], axis=0)
            res = _dot(dft_v[0:2 * _C, :], taps_t, _NT)
            for i, j in enumerate(chunks):
                t = res[:, _tile(i)]
                if j == 0:
                    t = jnp.concatenate([t[:_C] + dskip[:, _tile(g)], t[_C:]], axis=0)
                hf_v[j, :, :, :, _tile(g)] = t.reshape(2, FG, 8, 128)
            res = _dot(dft_v[3 * _C:5 * _C, :], shifted_kv(c, _tile(g)))
            for i, j in enumerate(chunks):
                xf_v[j, :, :, :, _tile(g)] = res[:, _tile(i)].reshape(2, FG, 8, 128)

    pins = []

    def chunk_conv(first, fg, g, zeros):
        half = NC // 2
        order = [k for i in range(half // 2) for k in (i, half - 1 - i)]

        def load(ref, imag, z):
            return ref[:, imag, (first + zeros[z]) + fg, :, _tile(g)]

        def pin(val):
            pins.append(None)
            yw_v[zeros[0] + (WT0 + D // 8 + len(pins) % 3), :, _tile(g)] = val

        def tri(a, b, i):
            acc = a[i] * b[0]
            for j in range(1, i + 1):
                acc = acc + a[i - j] * b[j]
            return acc

        def conv(a, b, emit):
            a, b = ([t[j] for j in range(NC)] for t in (a, b))
            part = {}
            for par in range(2):
                for i in order:
                    part[par, i] = tri(a[par::2], b[par::2], i)
                    pin(part[par, i])
                    yield 2 * i + 2
            sa, sb = ([t[2 * i] + t[2 * i + 1] for i in range(half)] for t in (a, b))
            for i in order:
                emit(2 * i, part[0, i] + part[1, i - 1] if i else part[0, i])
                emit(2 * i + 1, tri(sa, sb, i) - part[0, i] - part[1, i])
                yield 2 * i + 7

        common = {}

        def keep(i, t):
            common[i] = t
            pin(t)

        def real(i, t):
            yw_v[first + ((2 * i + 2) * FG + fg), :, _tile(g)] = common[i] - t

        def imag(i, t):
            yw_v[first + ((2 * i + 3) * FG + fg), :, _tile(g)] = common[i] + t

        yield from conv(load(xf_v, 0, 0) + load(xf_v, 1, 0), load(hf_v, 0, 0), keep)
        yield from conv(load(hf_v, 0, 1) + load(hf_v, 1, 1), load(xf_v, 1, 1), real)
        yield from conv(load(hf_v, 1, 2) - load(hf_v, 0, 2), load(xf_v, 0, 2), imag)

    def qv_proj(c, carry):
        n = FG // NQ
        zeros = [lax.shift_right_logical(c, 8 + i) for i in range(3)]
        work = (ops for i in range(n) for g in range(NG) for ops in chunk_conv(c * n, i, g, zeros))
        slots = 2 * D // 16
        per_slot = n * NG * 768 / (slots * NG + 3)
        budget = [0.0]

        def weights(cols):
            out = []
            for i in range(slots):
                while budget[0] > 0:
                    budget[0] -= next(work, budget[0])
                budget[0] += per_slot
                out.append(yw_v[WT0 + i, :, cols])
            return pltpu.bitcast(jnp.concatenate(out, axis=0), _BF16)

        def x_rows(j, m, cols):
            r0 = pl.multiple_of(c * (_QB // 2) + j * 64, 64)
            return pltpu.bitcast(xp_v[pl.ds(r0, m * 64), cols], _BF16)

        pj_v[...] = _dot(weights(_tile(NG - 1)), x_rows(0, NT, _tile(NG - 1)), _NT)
        for j in range(NT):
            r = _dot(weights(_tile(0, NG - 1)), x_rows(j, 1, _tile(0, NG - 1)), _NT)
            r = r + pj_v[:, _tile(j)]
            q_v[:, j, :, pl.ds(pl.multiple_of(c * 128, 128), 128)] = r[:D].reshape(D // 8, 8, 128)
            qb_v[pl.ds(pl.multiple_of(c * (D // 2), 8), D // 2), _tile(j)] = (
                pltpu.bitcast(r[:D].astype(_BF16), _U32))
            for h in range(0, _H, 2):
                t = r[D + h * Dh:D + (h + 2) * Dh]
                v_v[h * NQ + c, :, _tile(j)] = jnp.concatenate(
                    [t[:16], jnp.where(row < 4, t[16:24], 1.0)], axis=0)
                v_v[(h + 1) * NQ + c, :, _tile(j)] = jnp.concatenate(
                    [jnp.where(row < 4, 1.0, t[16:24]), t[24:]], axis=0)
        for _ in work:
            pass
        return carry

    lax.fori_loop(0, NQ, qv_proj, 0)

    def write_head(h, odd, qb, acc):
        den = acc[0:1] if odd else acc[_WIN - 1:_WIN]
        for j in range(NT):
            o_v[qb * NT + j, pl.ds(_aligned(h * _WIN, 8), _WIN), :] = acc[:, _tile(j)]
            den_v[qb * NT + j, pl.ds(h, 1), :] = den[:, _tile(j)]

    def q_window(h, qb):
        w = _aligned(qb * (D // 2) + ((Dh * h) >> 4) * 8, 8)
        return pltpu.bitcast(qb_v[pl.ds(w, _KWIN // 2), :], _BF16)

    def mxu_scores(h, qb, lo, n):
        keys = km_v[pl.ds(_aligned(4 * NM * h + 4 * lo, 8), 4 * n), :]
        return _dot(pltpu.bitcast(keys, _BF16)[:, :_KWIN], q_window(h, qb))

    def mxu_probs(h, qb, kc):
        lo, n = bounds[kc], bounds[kc + 1] - bounds[kc]
        p = jnp.exp2(mxu_scores(h, qb, lo, n))
        return {("m", lo + i): p[8 * i:8 * i + 8] for i in range(n)}

    def head_pair(i, carry):
        never = row > i + 8
        zero = lax.shift_right_logical(i, 8)
        probs = {("m", k): p_v[8 * k:8 * k + 8, :] for k in range(bounds[1])}
        s = None
        for odd in range(2):
            h = 2 * i + odd
            nxt = jnp.minimum(h + 1, _H - 2) if odd else h + 1
            spread_keys(nxt, 1 - odd, never)
            rows = [divmod(d + 4 * odd, 8) for d in range(Dh)]
            for qb in range(NQ):
                for kc in range(NK):
                    if kc + 1 < NK:
                        ahead = mxu_probs(h, qb, kc + 1)
                    elif qb + 1 < NQ:
                        ahead = mxu_probs(h, qb + 1, 0)
                    else:
                        ahead = mxu_probs(nxt, 0, 0)
                    for kind, idx in plan[kc]:
                        if kind == "m":
                            continue
                        zero = lax.shift_right_logical(zero, 1)
                        win = pl.ds(((Dh * h) >> 3) + zero, _WIN // 8)
                        q = [jnp.broadcast_to(q_v[win, :, lo:lo + 1, _tile(qb)],
                                              (_WIN // 8, NT, 8, 128)) for lo in range(8)]
                        keys = jnp.broadcast_to(kb_v[odd][zero, idx][:, None], (Dh, NT, 8, 128))
                        for d, (hi, lo) in enumerate(rows):
                            term = keys[d:d + 1] * q[lo][hi:hi + 1]
                            if d:
                                s = s + term
                            else:
                                s = term if s is None else jnp.where(never, s, term)
                        p = jnp.exp2(s).reshape(NT * 8, 128)
                        probs[kind, idx] = jnp.concatenate(
                            [p[8 * j:8 * j + 8] for j in range(NT)], axis=1)
                    tile = jnp.concatenate([probs.pop(key) for key in plan[kc][::-1]], axis=0)
                    r = _dot(v_v[h * NQ + kc // NT, :, _tile(kc % NT)], tile)
                    probs.update(ahead)
                    if kc == 0:
                        acc_v[...] = r
                    else:
                        acc = r + (acc_v[...] if kc == 1 else acc)
                write_head(h, odd, qb, acc)
        for k in range(bounds[1]):
            p_v[8 * k:8 * k + 8, :] = probs["m", k]
        return carry

    wo_cp.start()
    for (_, k), p in mxu_probs(0, 0, 0).items():
        p_v[8 * k:8 * k + 8, :] = p
    lax.fori_loop(0, _H // 2, head_pair, 0)

    den = den_v[...]
    safe = (den >= _DEN_RANGE[0]) & (den <= _DEN_RANGE[1])
    unsafe = jnp.max(jnp.max(jnp.where(safe, 0.0, 1.0), axis=0)).astype(jnp.int32)

    @pl.when(unsafe > 0)
    def _redo_with_true_row_max():
        def regroup(i, carry):
            r = pl.ds(pl.multiple_of(i * 8, 8), 8)
            for h in range(_H):
                kph_v[h, r, :] = head_cols(kp_v[r, :], h)
            return carry

        lax.fori_loop(0, NV, regroup, 0)

        def unit(u, carry):
            h, qb = u // NQ, u % NQ

            def scores(c):
                keys = kph_v[h, pl.ds(pl.multiple_of(c * (8 * NV // NQ), 8), 8 * NV // NQ), :]
                return {"m": mxu_scores(h, qb, c * (NM // NQ), NM // NQ),
                        "v": _dot(keys[:, :_KWIN], q_window(h, qb))}

            def running_max(c, m):
                for s in scores(c).values():
                    m = jnp.maximum(m, jnp.max(s, axis=0, keepdims=True))
                return m

            m = lax.fori_loop(0, NQ, running_max, jnp.full((1, _QB), -jnp.inf, _F32))

            def accumulate(c, acc):
                s = scores(c)
                p = [jnp.exp2(s[kind][8 * i:8 * i + 8] - m)
                     for kc in range(NK // NQ) for kind, i in plan[kc][::-1]]
                return acc + _dot(v_v[h * NQ + c], jnp.concatenate(p, axis=0))

            acc = lax.fori_loop(0, NQ, accumulate, jnp.zeros((_WIN, _QB), _F32))
            for odd in range(2):
                pl.when(h % 2 == odd)(lambda: write_head(h, odd, qb, acc))
            return carry

        lax.fori_loop(0, _H * NQ, unit, 0)

    wo_cp.wait()

    def finish(c, carry):
        for i in range(_FIN):
            j = c * _FIN + i
            out_rows = pl.ds(pl.multiple_of(j * _C, _C), _C)
            rcp_v[i] = jnp.concatenate([gt_v[j]] * (_H // 8), axis=0) / den_v[j]
            heads = []
            for h in range(0, _H, 2):
                e, f = (o_v[j, (h + u) * _WIN:(h + u + 1) * _WIN, :]
                        * jnp.broadcast_to(rcp_v[i, h + u:h + u + 1, :], (_WIN, 128))
                        for u in range(2))
                heads += [e[:16], jnp.where(row < 4, e[16:], f[:8]), f[8:]]
            o = jnp.concatenate(heads, axis=0).T.astype(_BF16)
            base = 2 * j * FG + lax.shift_right_logical(c, 8 + i % 2)
            res = []
            for g in range(NG):
                z = yw_v[pl.ds(base, 4 * FG), :, _tile(g)].reshape(8, _C // 2, 128)
                ar, br, ai, bi = z[4] - z[2], z[5] + z[3], z[6] + z[0], z[7] - z[1]
                for par in range(2):
                    lo = 2 * _C + par * _C // 2
                    y_v[i % 4 * NG + g, pl.ds(par, _C // 2, stride=2), :] = _dot(
                        dft_v[lo:lo + _C // 2, :],
                        jnp.concatenate((ar - br, ai + bi) if par else (ar + br, ai - bi), axis=0))
                res.append(_dot(o, wo_v[:, _tile(g)])
                           + xg_v[out_rows, _tile(g)] * y_v[i % 4 * NG + g])
            out_v[out_rows, :] = jnp.concatenate(res, axis=1).astype(out_v.dtype)
            pltpu.make_async_copy(out_v.at[out_rows], out_hbm.at[0, out_rows], osem).start()
        return carry

    lax.fori_loop(0, NC // _FIN, finish, 0)
    pltpu.make_async_copy(out_v, out_hbm.at[0], osem).wait()


@jax.jit
def pallas_gated_mix__mha_block__ssm_conv_h3__prompt_kernel(
    A_x: jax.Array,
    A_wqkv: jax.Array,
    A_wo: jax.Array,
    B_q: jax.Array,
    B_k: jax.Array,
    B_v: jax.Array,
    B_shift_k: jax.Array,
    B_ssm_k: jax.Array,
    B_ssm_D: jax.Array,
    gate_w: jax.Array,
):
    del B_q
    _, S, D = A_x.shape
    NQ, NC = S // _QB, S // _C
    _, _, NM, NV = _key_plan(S // _KC)
    hbm = pl.BlockSpec(memory_space=pl.ANY)
    vmem = pltpu.VMEM
    return pl.pallas_call(
        _kernel,
        out_shape=jax.ShapeDtypeStruct(A_x.shape, A_x.dtype),
        in_specs=[hbm] * 10,
        out_specs=hbm,
        scratch_shapes=[
            vmem((S // 2, D), _U32),
            vmem((S, D), _BF16),
            vmem((3, D, D), _BF16),
            vmem((D, D), _BF16),
            vmem((S, D), _BF16),
            vmem((S, D), _BF16),
            vmem((D, S), _BF16),
            vmem((_H * 4 * NM, 128), _U32),
            vmem((8 * NV, D), _F32),
            vmem((-(-8 * NV // 128), D, 128), _F32),
            vmem((_H, 8 * NV, 128), _F32),
            vmem((1, NV, D // _H, 8, 128), _F32),
            vmem((1, NV, D // _H, 8, 128), _F32),
            vmem((D // 8, _QB // 128, 8, (NQ + 1) * 128), _F32),
            vmem((NQ * D // 2, _QB), _U32),
            vmem((_H * NQ, _WIN, _QB), _F32),
            vmem((_KC, _QB), _F32),
            vmem((_WIN, _QB), _F32),
            vmem((S // 128, _H, 128), _F32),
            vmem((_FIN, _H, 128), _F32),
            vmem((S // 128, 8, 128), _F32),
            vmem((S, D), _F32),
            vmem((S // 128, _H * _WIN, 128), _F32),
            vmem((NC, 2, _C // 8, 8, D), _F32),
            vmem((NC, 2, _C // 8, 8, D), _F32),
            vmem(((S + _C) // 4 + D // 8 + 4, 8, D), _F32),
            vmem((2 * D, _QB), _F32),
            vmem((4 * D // 128, _C, 128), _F32),
            vmem((S, D), A_x.dtype),
            vmem((5 * _C, _C), _BF16),
            vmem(B_shift_k.shape[::-1], _BF16),
            vmem((D,), _BF16),
            vmem((D,), _BF16),
            pltpu.SemaphoreType.DMA((len(_X_CHUNKS) + 3 * len(_SSM_CHUNKS) + 4,)),
            pltpu.SemaphoreType.DMA(()),
        ],
        compiler_params=pltpu.CompilerParams(vmem_limit_bytes=122 * 1024 * 1024),
    )(A_x, A_wqkv, A_wo, B_k, B_v, B_ssm_k, B_shift_k.T, B_ssm_D, gate_w,
      _dft_matrices().astype(_BF16))
```
